```python
import jax
import jax.numpy as jnp

def _softmax(x, axis=-1):
    return jax.nn.softmax(x, axis=axis)
def _gelu(x):
    return jax.nn.gelu(x, approximate=True)
def _silu(x):
    return jax.nn.silu(x)
def _sigmoid(x):
    return jax.nn.sigmoid(x)
def _layernorm(x, axis=-1, eps=1e-5):
    m = jnp.mean(x, axis=axis, keepdims=True)
    v = jnp.var(x, axis=axis, keepdims=True)
    return (x - m) / jnp.sqrt(v + eps)
def _scatter_add(tgt, idx, src, axis=0):
    return tgt.at[idx].add(src)
def _segment_sum(src, seg, n):
    return jax.ops.segment_sum(src, seg, n)
class _Rng:
    def __init__(self, key):
        self._k = key
    def _next(self):
        self._k, sub = jax.random.split(self._k)
        return sub
    def normal(self, shape):
        return jax.random.normal(self._next(), shape, dtype=jnp.bfloat16)
    def randint(self, lo, hi, shape):
        return jax.random.randint(self._next(), shape, lo, hi, dtype=jnp.int32)
    def uniform(self, shape, lo=0.0, hi=1.0):
        return jax.random.uniform(self._next(), shape, jnp.bfloat16, lo, hi)
    def permutation(self, n):
        return jax.random.permutation(self._next(), n)


kernel_name = 'standalone__groupnorm__prompt'

def setup_inputs():
    _rng = _Rng(jax.random.key(int.from_bytes(__import__("os").urandom(4), "little")))
    _w = (lambda a: (lambda t: t.astype(jnp.bfloat16) if jnp.issubdtype(t.dtype, jnp.floating) else t)(jnp.asarray(a)))
    B = 2
    G = 32
    cpg = max(1, 1024 // G)
    C = G * cpg
    H, W = 32, 2048
    return {
        "x": _w((lambda *s: _rng.normal(s) * 0.05)(B, C, H, W)),
        "g": _w((lambda *s: _rng.normal(s) * 0.05)(C) + 1.0),
        "b": _w((lambda *s: _rng.normal(s) * 0.05)(C)),
    }

def reference(x, g, b):
    G = 32
    B, C, H, W = x.shape[0], x.shape[1], x.shape[2], x.shape[3]
    xr = x.reshape(B, G, C // G, H, W)
    mu = xr.mean(axis=(2, 3, 4), keepdims=True)
    var = ((xr - mu) ** 2).mean(axis=(2, 3, 4), keepdims=True)
    xn = (xr - mu) / jnp.sqrt(var + 1e-5)
    xn = xn.reshape(B, C, H, W)
    return xn * g[None, :, None, None] + b[None, :, None, None]
```

```python
import functools
import jax, jax.numpy as jnp
from jax import lax
from jax.experimental import pallas as pl
from jax.experimental.pallas import tpu as pltpu

G = 32
EPS = 1e-5
UNIT = 256


def make(phases=(24, 20, 20), rk=2, wG=4, wk=1, ahead=2, ov_rw=1, ov_wr=1, compute=True, r_alt=True, w_alt=False,
         unroll_rows=32, nacc=4, vmem_mb=120):
    def fn(x, g, b):
        B, C, H, W = x.shape
        cpg = C // G
        rows_g = cpg * H
        U = rows_g // UNIT
        NG = B * G
        NS = max(phases)
        assert sum(phases) == NG and all(p % wG == 0 for p in phases)
        nr = UNIT // (8 * rk)
        nw = UNIT // (8 * wk)
        n_el = rows_g * W
        cpu = UNIT // H

        def kern(x_hbm, g_hbm, b_hbm, o_hbm, buf, g_v, b_v, gb_f, gb_s, rsem, rtail, wsem, wtail, psem):
            def rd(grp, slot, q, sem):
                rs = pl.ds(q * rk * 8, rk * 8)
                return pltpu.make_async_copy(x_hbm.at[pl.ds(grp * U, U), rs], buf.at[pl.ds(slot * U, U), rs], sem)

            def wr(grp, slot, q, sem):
                rs = pl.ds(q * wk * 8, wk * 8)
                return pltpu.make_async_copy(buf.at[pl.ds(slot * U, wG * U), rs], o_hbm.at[pl.ds(grp * U, wG * U), rs], sem)

            def start_reads(grp, slot, tail=0):
                for q in range(nr):
                    rd(grp, slot, q, rtail if q >= nr - tail else rsem.at[slot]).start(priority=q % 2 if r_alt else 0)

            def start_writes(grp, slot, tail=0):
                for q in range(nw):
                    wr(grp, slot, q, wtail if q >= nw - tail else wsem.at[slot // wG]).start(priority=q % 2 if w_alt else 0)

            def process(grp, slot):
                if not compute:
                    return
                nstep = rows_g // unroll_rows
                spu = UNIT // unroll_rows

                def tile(i):
                    return buf.at[slot * U + i // spu, pl.ds(pl.multiple_of((i % spu) * unroll_rows, unroll_rows), unroll_rows)]

                def reduce_pass(f):
                    def body(i, accs):
                        accs = list(accs)
                        t = tile(i)
                        k = 0
                        for r in range(unroll_rows // 16):
                            for c in range(W // 128):
                                v = f(t[r * 16:(r + 1) * 16, c * 128:(c + 1) * 128].astype(jnp.float32))
                                accs[k % nacc] = accs[k % nacc] + v
                                k += 1
                        return tuple(accs)
                    accs = lax.fori_loop(0, nstep, body, tuple(jnp.zeros((16, 128), jnp.float32) for _ in range(nacc)))
                    tot = functools.reduce(lambda a, b_: a + b_, accs)
                    return jnp.sum(jnp.sum(tot, axis=0, keepdims=True), axis=1, keepdims=True)

                mu = reduce_pass(lambda v: v) * (1.0 / n_el)
                mu_b = jnp.broadcast_to(mu, (16, 128))
                var = reduce_pass(lambda v: (v - mu_b) * (v - mu_b)) * (1.0 / n_el)
                rstd = jnp.broadcast_to(lax.rsqrt(var + EPS), (16, 128))
                ch0 = (grp % G) * cpg

                def norm(c, _):
                    ch = ch0 + c
                    a = rstd * gb_s[0, ch // 128, ch % 128]
                    d = gb_s[1, ch // 128, ch % 128] - mu_b * a
                    t = buf.at[slot * U + c // cpu, pl.ds(pl.multiple_of((c % cpu) * H, H), H)]
                    for r in range(H // 16):
                        for cc in range(W // 128):
                            idx = (slice(r * 16, (r + 1) * 16), slice(cc * 128, (cc + 1) * 128))
                            t[idx] = (t[idx].astype(jnp.float32) * a + d).astype(jnp.bfloat16)
                lax.fori_loop(0, cpg, norm, None)

            for j in range(ahead):
                start_reads(j, j)
            cg = pltpu.make_async_copy(g_hbm, g_v, psem.at[0])
            cb = pltpu.make_async_copy(b_hbm, b_v, psem.at[1])
            cg.start(); cb.start(); cg.wait(); cb.wait()
            gb_f[0] = g_v[...].astype(jnp.float32).reshape(C // 128, 128)
            gb_f[1] = b_v[...].astype(jnp.float32).reshape(C // 128, 128)
            cs = pltpu.make_async_copy(gb_f, gb_s, psem.at[0])
            cs.start(); cs.wait()

            base = 0
            for ip, n in enumerate(phases):
                def rbody(j, _, base=base, n=n):
                    for q in range(nr):
                        rd(base + j, j, q, rsem.at[j]).wait()
                    @pl.when(j + ahead < n - 1)
                    def _():
                        start_reads(base + j + ahead, j + ahead)
                    @pl.when(j + ahead == n - 1)
                    def _():
                        start_reads(base + n - 1, n - 1, tail=ov_rw)
                    process(base + j, j)
                lax.fori_loop(0, n - 1, rbody, None)
                nb_ = n // wG
                for q in range(nr - ov_rw):
                    rd(base + n - 1, n - 1, q, rsem.at[n - 1]).wait()
                start_writes(base, 0)
                for q in range(nr - ov_rw, nr):
                    rd(base + n - 1, n - 1, q, rtail).wait()
                process(base + n - 1, n - 1)
                last = ip == len(phases) - 1
                def wbody(j, _, base=base):
                    start_writes(base + j * wG, j * wG)
                    for q in range(nw):
                        wr(base + (j - 1) * wG, (j - 1) * wG, q, wsem.at[j - 1]).wait()
                lax.fori_loop(1, nb_ - 1, wbody, None)
                tail = 0 if last else ov_wr
                start_writes(base + (nb_ - 1) * wG, (nb_ - 1) * wG, tail=tail)
                for q in range(nw):
                    wr(base + (nb_ - 2) * wG, (nb_ - 2) * wG, q, wsem.at[nb_ - 2]).wait()
                for q in range(nw - tail):
                    wr(base + (nb_ - 1) * wG, (nb_ - 1) * wG, q, wsem.at[nb_ - 1]).wait()
                if not last:
                    for j in range(ahead):
                        start_reads(base + n + j, j)
                for q in range(nw - tail, nw):
                    wr(base + (nb_ - 1) * wG, (nb_ - 1) * wG, q, wtail).wait()
                base += n

        shp = (NG * U, UNIT, W)
        return pl.pallas_call(
            kern,
            in_specs=[pl.BlockSpec(memory_space=pltpu.HBM)] * 3,
            out_specs=pl.BlockSpec(memory_space=pltpu.HBM),
            out_shape=jax.ShapeDtypeStruct(shp, x.dtype),
            scratch_shapes=[
                pltpu.VMEM((NS * U, UNIT, W), x.dtype),
                pltpu.VMEM((C,), g.dtype), pltpu.VMEM((C,), b.dtype),
                pltpu.VMEM((2, C // 128, 128), jnp.float32),
                pltpu.SMEM((2, C // 128, 128), jnp.float32),
                pltpu.SemaphoreType.DMA((NS,)), pltpu.SemaphoreType.DMA(()),
                pltpu.SemaphoreType.DMA((NS // wG,)), pltpu.SemaphoreType.DMA(()),
                pltpu.SemaphoreType.DMA((2,)),
            ],
            compiler_params=pltpu.CompilerParams(vmem_limit_bytes=vmem_mb * 2**20),
        )(x.reshape(shp), g, b).reshape(x.shape)
    return fn


@jax.jit
def pallas_standalone__groupnorm__prompt_kernel(x, g, b):
    return make()(x, g, b)
```

```python
import functools
import jax, jax.numpy as jnp
from jax import lax
from jax.experimental import pallas as pl
from jax.experimental.pallas import tpu as pltpu

G = 32
EPS = 1e-5
UNIT = 256
TR = UNIT // 8


def srl(v, n):
    assert n & (n - 1) == 0
    return lax.shift_right_logical(v, n.bit_length() - 1)


def make(nphase=3, rparts=((4, 0), (12, 1)), rp=4, wk=8, wp=8, lag=2, rt=1, wt=1, compute=True,
         its=(8, 8, 16), nacc=4, vmem_mb=120, wpre=2, ncomp=None):
    def fn(x, g, b):
        B, C, H, W = x.shape
        cpg = C // G
        rows_g = cpg * H
        U = rows_g // UNIT
        NG = B * G
        rk = sum(n for n, _ in rparts)
        rG = rk // U
        NB = NG // rG
        nmax = -(-NB // nphase)
        nbig = NB - (nmax - 1) * nphase
        rnc, wnc = 16 // rp, 16 // wp
        rsteps = TR * rnc
        tpg = rsteps // rG
        tpi = tpg // sum(its)
        assert tpi * sum(its) == tpg
        wpb = rk // wk
        assert wpb * wk == rk
        wrow_g = TR * U // wk
        n_el = rows_g * W
        VW = 256

        def kern(x_hbm, g_hbm, b_hbm, o_hbm, buf, g_v, b_v, gb_f, gb_s, rsem, wsem, psem):
            def read_step(base, n, j, t):
                q = srl(t, rnc)
                rs = pl.ds(pl.multiple_of(q * 8, 8), 8)
                cs = pl.ds(pl.multiple_of((t & (rnc - 1)) * (128 * rp), 128 * rp), 128 * rp)
                sem = rsem.at[jnp.where((j == n - 1) & (q >= TR - rt), nmax, j)]
                o = j * rk
                for cnt, prio in rparts:
                    pltpu.make_async_copy(x_hbm.at[pl.ds(base + o, cnt), rs, cs], buf.at[pl.ds(o, cnt), rs, cs], sem).start(priority=prio)
                    o = o + cnt

            def write_row(base, n, t):
                j, q = srl(t, TR), t & (TR - 1)
                rs = pl.ds(pl.multiple_of(q * 8, 8), 8)
                sem = wsem.at[jnp.where((j == n * wpb - 1) & (q >= TR - wt), nmax * wpb, j)]
                for c in range(wnc):
                    cs = pl.ds(c * 128 * wp, 128 * wp)
                    pltpu.make_async_copy(buf.at[pl.ds(j * wk, wk), rs, cs], o_hbm.at[pl.ds(base + j * wk, wk), rs, cs], sem).start()

            def wait(sem, u0, nu, q0, nq):
                if nq:
                    v = buf.at[pl.ds(u0, nu), pl.ds(q0 * 8, nq * 8)]
                    pltpu.make_async_copy(v, v, sem).wait()

            def process(grp, slot, tick):
                def tile(i, rows):
                    per = UNIT // rows
                    return buf.at[slot * U + srl(i, per), pl.ds(pl.multiple_of((i & (per - 1)) * rows, rows), rows)]

                def vregs(r0, rows):
                    return [(slice(r0 + r * 8, r0 + r * 8 + 8), slice(c * VW, (c + 1) * VW)) for r in range(rows // 8) for c in range(W // VW)]

                def reduce_pass(f, nit, t0):
                    rows = rows_g // nit
                    def body(i, accs):
                        tick(t0 + i)
                        accs = list(accs)
                        t = tile(i, rows)
                        for k, idx in enumerate(vregs(0, rows)):
                            accs[k % nacc] = accs[k % nacc] + f(t[idx].astype(jnp.float32))
                        return tuple(accs)
                    accs = lax.fori_loop(0, nit, body, tuple(jnp.zeros((8, VW), jnp.float32) for _ in range(nacc)))
                    v = functools.reduce(lambda a, b_: a + b_, accs)
                    return jnp.sum(jnp.sum(v, axis=0, keepdims=True), axis=1, keepdims=True)

                mu = jnp.broadcast_to(reduce_pass(lambda v: v, its[0], 0) * (1.0 / n_el), (8, VW))
                var = reduce_pass(lambda v: (v - mu) * (v - mu), its[1], its[0]) * (1.0 / n_el)
                rstd = jnp.broadcast_to(lax.rsqrt(var + EPS), (8, VW))
                ch0 = (grp & (G - 1)) * cpg
                nrows = rows_g // its[2]

                def norm(i, _):
                    tick(its[0] + its[1] + i)
                    t = tile(i, nrows)
                    for k in range(nrows // H):
                        ch = ch0 + i * (nrows // H) + k
                        hi, lo = srl(ch, 128), ch & 127
                        a = rstd * gb_s[0, hi, lo]
                        d = gb_s[1, hi, lo] - mu * a
                        for idx in vregs(k * H, H):
                            t[idx] = (t[idx].astype(jnp.float32) * a + d).astype(jnp.bfloat16)
                lax.fori_loop(0, its[2], norm, None)

            cg = pltpu.make_async_copy(g_hbm, g_v, psem.at[0])
            cb = pltpu.make_async_copy(b_hbm, b_v, psem.at[1])
            cs_ = pltpu.make_async_copy(gb_f, gb_s, psem.at[0])
            cg.start(); cb.start()

            def phase(ip, _):
                n = jnp.where(ip < nbig, nmax, nmax - 1)
                nprev = jnp.where(ip - 1 < nbig, nmax, nmax - 1)
                base = (ip * (nmax - 1) + jnp.minimum(ip, nbig)) * rk
                gbase = srl(base, U)
                nc = n - lag if ncomp is None else ncomp

                def issue(t, _):
                    read_step(base, n, srl(t, rsteps), t & (rsteps - 1))
                lax.fori_loop(0, rsteps, issue, None, unroll=2)

                @pl.when(ip == 0)
                def _():
                    cg.wait(); cb.wait()
                    gb_f[0] = g_v[...].astype(jnp.float32).reshape(C // 128, 128)
                    gb_f[1] = b_v[...].astype(jnp.float32).reshape(C // 128, 128)
                    cs_.start()

                @pl.when(ip > 0)
                def _():
                    wait(wsem.at[nmax * wpb], nprev * rk - wk, wk, TR - wt, wt)
                lax.fori_loop(rsteps, (n - nc) * rsteps, issue, None)

                @pl.when(ip == 0)
                def _():
                    cs_.wait()

                def rgroup(s, _):
                    j, k = srl(s, rG), s & (rG - 1)
                    @pl.when(k == 0)
                    def _():
                        wait(rsem.at[j], j * rk, rk, 0, TR)
                    def tick(i):
                        for u in range(tpi):
                            read_step(base, n, j + n - nc, k * tpg + i * tpi + u)
                    if compute:
                        process(gbase + s, s, tick)
                    else:
                        lax.fori_loop(0, sum(its), lambda i, _: tick(i), None)
                lax.fori_loop(0, nc * rG, rgroup, None)

                lax.fori_loop(nc, n - 1, lambda j, _: wait(rsem.at[j], j * rk, rk, 0, TR), None)
                wait(rsem.at[n - 1], (n - 1) * rk, rk, 0, TR - rt)
                wissue = lambda t, _: write_row(base, n, t)
                lax.fori_loop(0, wpre * wrow_g, wissue, None)
                wait(rsem.at[nmax], (n - 1) * rk, rk, TR - rt, rt)

                def wgroup(i, _):
                    s = nc * rG + i
                    if compute:
                        process(gbase + s, s, lambda i: None)
                    lax.fori_loop((wpre + i) * wrow_g, (wpre + i + 1) * wrow_g, wissue, None)
                lax.fori_loop(0, (n - nc) * rG, wgroup, None)
                lax.fori_loop((wpre + (n - nc) * rG) * wrow_g, n * rG * wrow_g, wissue, None)
                lax.fori_loop(0, n * wpb - 1, lambda j, _: wait(wsem.at[j], j * wk, wk, 0, TR), None)
                wait(wsem.at[n * wpb - 1], n * rk - wk, wk, 0, TR - wt)
            lax.fori_loop(0, nphase, phase, None)
            nlast = nmax if nphase - 1 < nbig else nmax - 1
            wait(wsem.at[nmax * wpb], nlast * rk - wk, wk, TR - wt, wt)

        shp = (NG * U, UNIT, W)
        return pl.pallas_call(
            kern,
            in_specs=[pl.BlockSpec(memory_space=pltpu.HBM)] * 3,
            out_specs=pl.BlockSpec(memory_space=pltpu.HBM),
            out_shape=jax.ShapeDtypeStruct(shp, x.dtype),
            scratch_shapes=[
                pltpu.VMEM((nmax * rk, UNIT, W), x.dtype),
                pltpu.VMEM((C,), g.dtype), pltpu.VMEM((C,), b.dtype),
                pltpu.VMEM((2, C // 128, 128), jnp.float32),
                pltpu.SMEM((2, C // 128, 128), jnp.float32),
                pltpu.SemaphoreType.DMA((nmax + 1,)),
                pltpu.SemaphoreType.DMA((nmax * wpb + 1,)),
                pltpu.SemaphoreType.DMA((2,)),
            ],
            compiler_params=pltpu.CompilerParams(vmem_limit_bytes=vmem_mb * 2**20),
        )(x.reshape(shp), g, b).reshape(x.shape)
    return fn


@jax.jit
def pallas_standalone__groupnorm__prompt_kernel(x, g, b):
    return make()(x, g, b)
```

```python
import jax
import jax.numpy as jnp
from jax import lax
import jax.experimental.pallas as pl
import jax.experimental.pallas.tpu as pltpu

_GROUPS = 32
_EPS = 1e-5

_TILE = 8
_UNIT_ROWS = 256
_BATCH_UNITS = 16
_READ_SPLIT = ((13, 1), (3, 0))
_READ_COLS = 256
_WRITE_COLS = 1024
_PHASES = 3
_ITERS = (8, 8, 16)


def _div(v, n):
    assert n & (n - 1) == 0
    return lax.shift_right_logical(v, n.bit_length() - 1)


def _mod(v, n):
    assert n & (n - 1) == 0
    return v & (n - 1)


def _ds(index, size):
    return pl.ds(pl.multiple_of(index * size, size), size)


def _for(lo, hi, body):
    lax.fori_loop(lo, hi, lambda i, _: body(i), None)


def groupnorm(x, g, b, **call_kwargs):
    B, C, H, W = x.shape
    channels = C // _GROUPS
    group_rows = channels * H
    group_units = group_rows // _UNIT_ROWS
    n_units = B * _GROUPS * group_units
    tile_rows = _UNIT_ROWS // _TILE
    batch_groups = _BATCH_UNITS // group_units
    n_batches = n_units // _BATCH_UNITS
    max_batches = pl.cdiv(n_batches, _PHASES)
    n_long = n_batches - (max_batches - 1) * _PHASES
    read_steps = W // _READ_COLS
    ticks = sum(_ITERS)
    overlap_rows = 2 * tile_rows
    tick_reads = overlap_rows * read_steps // (batch_groups * ticks)

    assert group_units * _UNIT_ROWS == group_rows
    assert batch_groups * group_units == _BATCH_UNITS
    assert n_batches * _BATCH_UNITS == n_units and max_batches >= 5
    assert sum(n for n, _ in _READ_SPLIT) == _BATCH_UNITS
    assert tick_reads * batch_groups * ticks == overlap_rows * read_steps
    assert read_steps % tick_reads == 0
    assert _BATCH_UNITS >= group_units + 2 * max_batches

    def kernel(x_hbm, g_hbm, b_hbm, o_hbm, buf, g_vmem, b_vmem, gb_vmem, gb_smem,
               read_sems, write_sems, param_sems):
        read_tail, write_tail = max_batches, _BATCH_UNITS

        def phase_extent(p):
            first = p * (max_batches - 1) + jnp.minimum(p, n_long)
            return (first * _BATCH_UNITS,
                    jnp.where(p < n_long, max_batches, max_batches - 1))

        def read_copy(base, unit, n, rows, cols, sem):
            return pltpu.make_async_copy(
                x_hbm.at[pl.ds(base + unit, n), rows, cols],
                buf.at[pl.ds(unit, n), rows, cols], read_sems.at[sem])

        def on_write_copy(action, base, n, window, rows, cols, sem):
            for units in (max_batches, max_batches - 1):
                @pl.when(n == units)
                def _():
                    action(pltpu.make_async_copy(
                        buf.at[pl.ds(window * units, units), rows, cols],
                        o_hbm.at[pl.ds(base + window * units, units), rows, cols],
                        write_sems.at[sem]))

        all_rows, all_cols = pl.ds(0, _UNIT_ROWS), pl.ds(0, W)
        head_rows = pl.ds(0, _UNIT_ROWS - _TILE)
        tail_rows = pl.ds(_UNIT_ROWS - _TILE, _TILE)

        def wait_write_tail(p):
            on_write_copy(lambda copy: copy.wait(), *phase_extent(p),
                          _BATCH_UNITS - 1, tail_rows, all_cols, write_tail)

        def normalise(group, slot, tick=lambda i: None, before_pass=lambda k: None):
            def block(i, rows):
                per_unit = _UNIT_ROWS // rows
                return buf.at[slot * group_units + _div(i, per_unit),
                              _ds(_mod(i, per_unit), rows)]

            def mean_of(f, trips, first_tick):
                rows = group_rows // trips

                def body(i, acc):
                    tick(first_tick + i)
                    ref = block(i, rows)
                    for r in range(0, rows, _TILE):
                        acc = acc + f(ref[r:r + _TILE].astype(jnp.float32))
                    return acc

                acc = lax.fori_loop(0, trips, body, jnp.zeros((_TILE, W), jnp.float32))
                total = jnp.sum(jnp.sum(acc, axis=1, keepdims=True), axis=0, keepdims=True)
                return total * (1.0 / (group_rows * W))

            before_pass(0)
            mean = mean_of(lambda v: v, _ITERS[0], 0)
            before_pass(1)
            var = mean_of(lambda v: (v - mean) * (v - mean), _ITERS[1], _ITERS[0])
            rstd = lax.rsqrt(var + _EPS)
            per_trip = channels // _ITERS[2]

            def apply(i):
                tick(_ITERS[0] + _ITERS[1] + i)
                ref = block(i, per_trip * H)
                for k in range(per_trip):
                    c = _mod(group, _GROUPS) * channels + i * per_trip + k
                    scale = rstd * gb_smem[0, _div(c, 128), _mod(c, 128)]
                    shift = gb_smem[1, _div(c, 128), _mod(c, 128)] - mean * scale
                    for r in range(k * H, (k + 1) * H, _TILE):
                        v = ref[r:r + _TILE].astype(jnp.float32)
                        ref[r:r + _TILE] = (v * scale + shift).astype(buf.dtype)

            before_pass(2)
            _for(0, _ITERS[2], apply)

        g_copy = pltpu.make_async_copy(g_hbm, g_vmem, param_sems.at[0])
        b_copy = pltpu.make_async_copy(b_hbm, b_vmem, param_sems.at[1])
        gb_copy = pltpu.make_async_copy(gb_vmem, gb_smem, param_sems.at[2])
        g_copy.start()
        b_copy.start()

        def run_phase(p):
            base, n = phase_extent(p)
            first_group = _div(base, group_units)
            n_groups = n * batch_groups
            last_row = n * tile_rows - 1

            def start_reads(row, chunk, n_steps):
                batch = _div(row, tile_rows)
                sem = jnp.where(row == last_row, read_tail, batch)
                index = (_ds(_mod(row, tile_rows), _TILE),
                         all_cols if n_steps == read_steps
                         else _ds(chunk, n_steps * _READ_COLS))
                src = x_hbm.at[pl.ds(base + batch * _BATCH_UNITS, _BATCH_UNITS), *index]
                dst = buf.at[pl.ds(batch * _BATCH_UNITS, _BATCH_UNITS), *index]
                for step in range(n_steps):
                    unit = 0
                    for count, priority in _READ_SPLIT:
                        piece = (pl.ds(unit, count), slice(None),
                                 pl.ds(step * _READ_COLS, _READ_COLS))
                        pltpu.make_async_copy(
                            src.at[piece], dst.at[piece], read_sems.at[sem]
                        ).start(priority=priority)
                        unit += count

            def read_row(row):
                start_reads(row, 0, read_steps)

            def wait_batch(batch, rows=all_rows, sem=None):
                read_copy(base, batch * _BATCH_UNITS, _BATCH_UNITS, rows, all_cols,
                          batch if sem is None else sem).wait()

            _for(0, tile_rows, read_row)

            @pl.when(p == 0)
            def _():
                g_copy.wait()
                b_copy.wait()
                gb_vmem[0] = g_vmem[...].astype(jnp.float32).reshape(C // 128, 128)
                gb_vmem[1] = b_vmem[...].astype(jnp.float32).reshape(C // 128, 128)
                gb_copy.start()

            @pl.when(p > 0)
            def _():
                wait_write_tail(p - 1)

            overlap_start = last_row - overlap_rows
            _for(tile_rows, overlap_start, read_row)

            @pl.when(p == 0)
            def _():
                gb_copy.wait()

            wait_batch(0)

            def group_under_reads(slot):
                def tick(i):
                    k = slot * ticks + i
                    chunks = read_steps // tick_reads
                    start_reads(overlap_start + _div(k, chunks), _mod(k, chunks),
                                tick_reads)

                normalise(first_group + slot, slot, tick)

            _for(0, batch_groups, group_under_reads)
            read_row(last_row)
            _for(1, n - 1, wait_batch)
            wait_batch(n - 1, head_rows)

            write_rows = _BATCH_UNITS * tile_rows
            rows_per_group = lax.div(group_units * tile_rows, n)

            def write_row(row):
                window = _div(row, tile_rows)
                sem = jnp.where(row == write_rows - 1, write_tail, window)
                for col in range(0, W, _WRITE_COLS):
                    on_write_copy(lambda copy: copy.start(), base, n, window,
                                  _ds(_mod(row, tile_rows), _TILE),
                                  pl.ds(col, _WRITE_COLS), sem)

            def wait_window(window, rows=all_rows):
                on_write_copy(lambda copy: copy.wait(), base, n, window, rows,
                              all_cols, window)

            _for(0, rows_per_group, write_row)
            wait_batch(n - 1, tail_rows, read_tail)

            def group_under_writes(slot):
                first_row = (slot - batch_groups + 1) * rows_per_group

                def before_pass(k):
                    _for(first_row + lax.div(k * rows_per_group, 3),
                         first_row + lax.div((k + 1) * rows_per_group, 3), write_row)

                normalise(first_group + slot, slot, before_pass=before_pass)

            _for(batch_groups, n_groups, group_under_writes)
            _for((n_groups - batch_groups + 1) * rows_per_group, write_rows, write_row)
            _for(0, _BATCH_UNITS - 1, wait_window)
            wait_window(_BATCH_UNITS - 1, head_rows)

        _for(0, _PHASES, run_phase)
        wait_write_tail(_PHASES - 1)

    shape = (n_units, _UNIT_ROWS, W)
    hbm = pl.BlockSpec(memory_space=pltpu.HBM)
    out = pl.pallas_call(
        kernel,
        in_specs=[hbm, hbm, hbm],
        out_specs=hbm,
        out_shape=jax.ShapeDtypeStruct(shape, x.dtype),
        scratch_shapes=[
            pltpu.VMEM((max_batches * _BATCH_UNITS, _UNIT_ROWS, W), x.dtype),
            pltpu.VMEM((C,), g.dtype),
            pltpu.VMEM((C,), b.dtype),
            pltpu.VMEM((2, C // 128, 128), jnp.float32),
            pltpu.SMEM((2, C // 128, 128), jnp.float32),
            pltpu.SemaphoreType.DMA((max_batches + 1,)),
            pltpu.SemaphoreType.DMA((_BATCH_UNITS + 1,)),
            pltpu.SemaphoreType.DMA((3,)),
        ],
        compiler_params=pltpu.CompilerParams(vmem_limit_bytes=112 * 1024 * 1024),
        **call_kwargs,
    )(x.reshape(shape), g, b)
    return out.reshape(x.shape)


@jax.jit
def pallas_standalone__groupnorm__prompt_kernel(
    x: jax.Array,
    g: jax.Array,
    b: jax.Array,
):
    return groupnorm(x, g, b)
```

```python
import jax
import jax.numpy as jnp
from jax import lax
import jax.experimental.pallas as pl
import jax.experimental.pallas.tpu as pltpu

_GROUPS = 32
_EPS = 1e-5

_TILE = 8
_UNIT_ROWS = 256
_BATCH_UNITS = 16
_READ_SPLIT = ((13, 1), (3, 0))
_READ_COLS = 256
_WRITE_COLS = 1024
_PHASES = 3
_ITERS = (8, 8, 16)


def _div(v, n):
    assert n & (n - 1) == 0
    return lax.shift_right_logical(v, n.bit_length() - 1)


def _mod(v, n):
    assert n & (n - 1) == 0
    return v & (n - 1)


def _ds(index, size):
    return pl.ds(pl.multiple_of(index * size, size), size)


def _for(lo, hi, body):
    lax.fori_loop(lo, hi, lambda i, _: body(i), None)


def groupnorm(x, g, b, **call_kwargs):
    B, C, H, W = x.shape
    channels = C // _GROUPS
    group_rows = channels * H
    group_units = group_rows // _UNIT_ROWS
    n_units = B * _GROUPS * group_units
    tile_rows = _UNIT_ROWS // _TILE
    batch_groups = _BATCH_UNITS // group_units
    n_batches = n_units // _BATCH_UNITS
    max_batches = pl.cdiv(n_batches, _PHASES)
    n_long = n_batches - (max_batches - 1) * _PHASES
    read_steps = W // _READ_COLS
    ticks = sum(_ITERS)
    overlap_rows = 2 * tile_rows
    tick_reads = overlap_rows * read_steps // (batch_groups * ticks)

    assert group_units * _UNIT_ROWS == group_rows
    assert batch_groups * group_units == _BATCH_UNITS
    assert n_batches * _BATCH_UNITS == n_units and max_batches >= 5
    assert sum(n for n, _ in _READ_SPLIT) == _BATCH_UNITS
    assert tick_reads * batch_groups * ticks == overlap_rows * read_steps
    assert read_steps % tick_reads == 0
    assert (batch_groups - 2) * group_units >= max_batches

    def kernel(x_hbm, g_hbm, b_hbm, o_hbm, buf, g_vmem, b_vmem, gb_vmem, gb_smem,
               read_sems, write_sems, param_sems):
        read_tail, write_tail = max_batches, _BATCH_UNITS

        def phase_extent(p):
            first = p * (max_batches - 1) + jnp.minimum(p, n_long)
            return (first * _BATCH_UNITS,
                    jnp.where(p < n_long, max_batches, max_batches - 1))

        def read_copy(base, unit, n, rows, cols, sem):
            return pltpu.make_async_copy(
                x_hbm.at[pl.ds(base + unit, n), rows, cols],
                buf.at[pl.ds(unit, n), rows, cols], read_sems.at[sem])

        def on_write_copy(action, base, n, window, rows, cols, sem):
            for units in (max_batches, max_batches - 1):
                @pl.when(n == units)
                def _():
                    action(pltpu.make_async_copy(
                        buf.at[pl.ds(window * units, units), rows, cols],
                        o_hbm.at[pl.ds(base + window * units, units), rows, cols],
                        write_sems.at[sem]))

        all_rows, all_cols = pl.ds(0, _UNIT_ROWS), pl.ds(0, W)
        head_rows = pl.ds(0, _UNIT_ROWS - _TILE)
        tail_rows = pl.ds(_UNIT_ROWS - _TILE, _TILE)

        def wait_write_tail(p):
            on_write_copy(lambda copy: copy.wait(), *phase_extent(p),
                          _BATCH_UNITS - 1, tail_rows, all_cols, write_tail)

        def normalise(group, slot, tick=lambda i: None, before_pass=lambda k: None):
            def block(i, rows):
                per_unit = _UNIT_ROWS // rows
                return buf.at[slot * group_units + _div(i, per_unit),
                              _ds(_mod(i, per_unit), rows)]

            def mean_of(f, trips, first_tick):
                rows = group_rows // trips

                def body(i, acc):
                    tick(first_tick + i)
                    ref = block(i, rows)
                    for r in range(0, rows, _TILE):
                        acc = acc + f(ref[r:r + _TILE].astype(jnp.float32))
                    return acc

                acc = lax.fori_loop(0, trips, body, jnp.zeros((_TILE, W), jnp.float32))
                total = jnp.sum(jnp.sum(acc, axis=1, keepdims=True), axis=0, keepdims=True)
                return total * (1.0 / (group_rows * W))

            before_pass(0)
            mean = mean_of(lambda v: v, _ITERS[0], 0)
            before_pass(1)
            var = mean_of(lambda v: (v - mean) * (v - mean), _ITERS[1], _ITERS[0])
            rstd = lax.rsqrt(var + _EPS)
            per_trip = channels // _ITERS[2]

            def apply(i):
                tick(_ITERS[0] + _ITERS[1] + i)
                ref = block(i, per_trip * H)
                for k in range(per_trip):
                    c = _mod(group, _GROUPS) * channels + i * per_trip + k
                    scale = rstd * gb_smem[0, _div(c, 128), _mod(c, 128)]
                    shift = gb_smem[1, _div(c, 128), _mod(c, 128)] - mean * scale
                    for r in range(k * H, (k + 1) * H, _TILE):
                        v = ref[r:r + _TILE].astype(jnp.float32)
                        ref[r:r + _TILE] = (v * scale + shift).astype(buf.dtype)

            before_pass(2)
            _for(0, _ITERS[2], apply)

        g_copy = pltpu.make_async_copy(g_hbm, g_vmem, param_sems.at[0])
        b_copy = pltpu.make_async_copy(b_hbm, b_vmem, param_sems.at[1])
        gb_copy = pltpu.make_async_copy(gb_vmem, gb_smem, param_sems.at[2])
        g_copy.start()
        b_copy.start()

        def run_phase(p):
            base, n = phase_extent(p)
            first_group = _div(base, group_units)
            n_groups = n * batch_groups
            last_row = n * tile_rows - 1

            def start_reads(row, chunk, n_steps):
                batch = _div(row, tile_rows)
                sem = jnp.where(row == last_row, read_tail, batch)
                rows = _ds(_mod(row, tile_rows), _TILE)
                cols = (all_cols if n_steps == read_steps
                        else _ds(chunk, n_steps * _READ_COLS))
                src = x_hbm.at[pl.ds(base + batch * _BATCH_UNITS, _BATCH_UNITS), rows, cols]
                dst = buf.at[pl.ds(batch * _BATCH_UNITS, _BATCH_UNITS), rows, cols]
                for step in range(n_steps):
                    unit = 0
                    for count, priority in _READ_SPLIT:
                        piece = (pl.ds(unit, count), slice(None),
                                 pl.ds(step * _READ_COLS, _READ_COLS))
                        pltpu.make_async_copy(
                            src.at[piece], dst.at[piece], read_sems.at[sem]
                        ).start(priority=priority)
                        unit += count

            def read_row(row):
                start_reads(row, 0, read_steps)

            def wait_batch(batch, rows=all_rows, sem=None):
                read_copy(base, batch * _BATCH_UNITS, _BATCH_UNITS, rows, all_cols,
                          batch if sem is None else sem).wait()

            _for(0, tile_rows, read_row)

            @pl.when(p == 0)
            def _():
                g_copy.wait()
                b_copy.wait()
                gb_vmem[0] = g_vmem[...].astype(jnp.float32).reshape(C // 128, 128)
                gb_vmem[1] = b_vmem[...].astype(jnp.float32).reshape(C // 128, 128)
                gb_copy.start()

            @pl.when(p > 0)
            def _():
                wait_write_tail(p - 1)

            overlap_start = last_row - overlap_rows
            _for(tile_rows, overlap_start, read_row)

            @pl.when(p == 0)
            def _():
                gb_copy.wait()

            wait_batch(0)

            def group_under_reads(slot):
                def tick(i):
                    k = slot * ticks + i
                    chunks = read_steps // tick_reads
                    start_reads(overlap_start + _div(k, chunks), _mod(k, chunks),
                                tick_reads)

                normalise(first_group + slot, slot, tick)

            _for(0, batch_groups, group_under_reads)
            read_row(last_row)
            _for(1, n - 1, wait_batch)
            wait_batch(n - 1, head_rows)

            write_rows = _BATCH_UNITS * tile_rows
            rows_per_group = lax.div(group_units * tile_rows, n)

            def write_row(row):
                window = _div(row, tile_rows)
                sem = jnp.where(row == write_rows - 1, write_tail, window)
                for col in range(0, W, _WRITE_COLS):
                    on_write_copy(lambda copy: copy.start(), base, n, window,
                                  _ds(_mod(row, tile_rows), _TILE),
                                  pl.ds(col, _WRITE_COLS), sem)

            def wait_window(window, rows=all_rows):
                on_write_copy(lambda copy: copy.wait(), base, n, window, rows,
                              all_cols, window)

            _for(0, rows_per_group, write_row)
            wait_batch(n - 1, tail_rows, read_tail)

            def group_under_writes(slot):
                first_row = (slot - batch_groups + 1) * rows_per_group

                def before_pass(k):
                    _for(first_row + lax.div(k * rows_per_group, 3),
                         first_row + lax.div((k + 1) * rows_per_group, 3), write_row)

                normalise(first_group + slot, slot, before_pass=before_pass)

            _for(batch_groups, n_groups, group_under_writes)
            _for((n_groups - batch_groups + 1) * rows_per_group, write_rows, write_row)
            _for(0, _BATCH_UNITS - 1, wait_window)
            wait_window(_BATCH_UNITS - 1, head_rows)

        _for(0, _PHASES, run_phase)
        wait_write_tail(_PHASES - 1)

    shape = (n_units, _UNIT_ROWS, W)
    hbm = pl.BlockSpec(memory_space=pltpu.HBM)
    out = pl.pallas_call(
        kernel,
        in_specs=[hbm, hbm, hbm],
        out_specs=hbm,
        out_shape=jax.ShapeDtypeStruct(shape, x.dtype),
        scratch_shapes=[
            pltpu.VMEM((max_batches * _BATCH_UNITS, _UNIT_ROWS, W), x.dtype),
            pltpu.VMEM((C,), g.dtype),
            pltpu.VMEM((C,), b.dtype),
            pltpu.VMEM((2, C // 128, 128), jnp.float32),
            pltpu.SMEM((2, C // 128, 128), jnp.float32),
            pltpu.SemaphoreType.DMA((max_batches + 1,)),
            pltpu.SemaphoreType.DMA((_BATCH_UNITS + 1,)),
            pltpu.SemaphoreType.DMA((3,)),
        ],
        compiler_params=pltpu.CompilerParams(vmem_limit_bytes=112 * 1024 * 1024),
        **call_kwargs,
    )(x.reshape(shape), g, b)
    return out.reshape(x.shape)


@jax.jit
def pallas_standalone__groupnorm__prompt_kernel(
    x: jax.Array,
    g: jax.Array,
    b: jax.Array,
):
    return groupnorm(x, g, b)
```
